```python
import os as _os
_os.environ.setdefault("JAX_PLATFORMS", "cpu")
import jax
import jax.numpy as jnp

def _softmax(x, axis=-1):
    return jax.nn.softmax(x, axis=axis)
def _gelu(x):
    return jax.nn.gelu(x, approximate=True)
def _silu(x):
    return jax.nn.silu(x)
def _sigmoid(x):
    return jax.nn.sigmoid(x)
def _layernorm(x, axis=-1, eps=1e-5):
    m = jnp.mean(x, axis=axis, keepdims=True)
    v = jnp.var(x, axis=axis, keepdims=True)
    return (x - m) / jnp.sqrt(v + eps)
def _scatter_add(tgt, idx, src, axis=0):
    return tgt.at[idx].add(src)
def _segment_sum(src, seg, n):
    return jax.ops.segment_sum(src, seg, n)
class _Rng:
    def __init__(self, key):
        self._k = key
    def _next(self):
        self._k, sub = jax.random.split(self._k)
        return sub
    def normal(self, shape):
        return jax.random.normal(self._next(), shape, dtype=jnp.bfloat16)
    def randint(self, lo, hi, shape):
        return jax.random.randint(self._next(), shape, lo, hi, dtype=jnp.int32)
    def uniform(self, shape, lo=0.0, hi=1.0):
        return jax.random.uniform(self._next(), shape, jnp.bfloat16, lo, hi)
    def permutation(self, n):
        return jax.random.permutation(self._next(), n)


kernel_name = 'interleave_layers__sliding_local_dilated__linear_kernel_hedgehog__prompt'

def setup_inputs():
    _rng = _Rng(jax.random.key(int.from_bytes(__import__("os").urandom(4), "little")))
    _w = (lambda a: (lambda t: t.astype(jnp.bfloat16) if jnp.issubdtype(t.dtype, jnp.floating) else t)(jnp.asarray(a)))
    def _A_setup():
        B, S, D = 1, 2048, 640
        return {
            "x": _w((lambda *s: _rng.normal(s) * 0.05)(B, S, D)),
            "wqkv": _w((lambda *s: _rng.normal(s) * 0.05)(D, 3 * D)),
            "wo": _w((lambda *s: _rng.normal(s) * 0.05)(D, D)),
        }
    _A_in = _A_setup()

    def _B_setup():
        B, S, D, H = 1, 2048, 640, 32
        Dh = D // H
        return {
            "x": _w((lambda *s: _rng.normal(s) * 0.05)(B, S, D)),
            "wqkv": _w((lambda *s: _rng.normal(s) * 0.4)(D, 3 * D)),
            "w_phi": _w((lambda *s: _rng.normal(s) * 0.4)(H, Dh, Dh) * (Dh ** -0.5)),
            "wo": _w((lambda *s: _rng.normal(s) * 0.1)(D, D)),
        }
    _B_in = _B_setup()

    return {
        "A_x": _A_in["x"],
        "A_wqkv": _A_in["wqkv"],
        "A_wo": _A_in["wo"],
        "B_x": _B_in["x"],
        "B_wqkv": _B_in["wqkv"],
        "B_w_phi": _B_in["w_phi"],
        "B_wo": _B_in["wo"],
    }

def reference(A_x, A_wqkv, A_wo, B_x, B_wqkv, B_w_phi, B_wo):
    def _A_ref(x, wqkv, wo):
        B, S, D = x.shape
        H = 32; Dh = D // H
        W, dil = 8, 2
        qkv = (lambda x, *d: x.transpose(*d))((x @ wqkv).reshape(B, S, 3, H, Dh), 2, 0, 3, 1, 4)
        q, k, v = qkv[0], qkv[1], qkv[2]
        scale = Dh ** -0.5
        pos = jnp.arange(S)
        off = jnp.arange(W) * dil
        idx = pos[:, None] - off[None, :]
        mask = idx >= 0
        idx_c = jnp.where(mask, idx, 0).reshape(-1)
        kg = k[:, :, idx_c, :].reshape(B, H, S, W, Dh)
        vg = v[:, :, idx_c, :].reshape(B, H, S, W, Dh)
        logits = jnp.einsum("bhsd,bhswd->bhsw", q, kg) * scale
        logits = jnp.where(mask[None, None, :, :], logits, -1e9)
        attn = _softmax(logits, axis=-1)
        o = jnp.einsum("bhsw,bhswd->bhsd", attn, vg)
        return (lambda x, *d: x.transpose(*d))(o, 0, 2, 1, 3).reshape(B, S, D) @ wo

    def _B_ref(x, wqkv, w_phi, wo):
        B, S, D = x.shape
        H = 32; Dh = D // H
        qkv = (lambda x, *d: x.transpose(*d))((x @ wqkv).reshape(B, S, 3, H, Dh), 2, 0, 3, 1, 4)
        q, k, v = qkv[0], qkv[1], qkv[2]
        pq = jnp.einsum("bhsd,hdf->bhsf", q, w_phi)
        pk = jnp.einsum("bhsd,hdf->bhsf", k, w_phi)
        phi_q = jnp.concatenate([_softmax(pq, axis=-1), _softmax(-pq, axis=-1)], axis=-1)
        phi_k = jnp.concatenate([_softmax(pk, axis=-1), _softmax(-pk, axis=-1)], axis=-1)
        kv = jnp.einsum("bhsf,bhsd->bhfd", phi_k, v)
        z  = jnp.einsum("bhsf->bhf", phi_k)
        num = jnp.einsum("bhqf,bhfd->bhqd", phi_q, kv)
        den = jnp.einsum("bhqf,bhf->bhq", phi_q, z)[..., None] + 1e-6
        o = num / den
        return (lambda x, *d: x.transpose(*d))(o, 0, 2, 1, 3).reshape(B, S, D) @ wo

    x = A_x
    x = x + _A_ref(_layernorm(x, axis=-1), A_wqkv, A_wo)
    x = x + _B_ref(_layernorm(x, axis=-1), B_wqkv, B_w_phi, B_wo)
    x = x + _A_ref(_layernorm(x, axis=-1), A_wqkv, A_wo)
    x = x + _B_ref(_layernorm(x, axis=-1), B_wqkv, B_w_phi, B_wo)
    return x
```

```python
import jax
import jax.numpy as jnp
from jax import lax
import jax.experimental.pallas as pl
import jax.experimental.pallas.tpu as pltpu

S, D, H, DH = 2048, 640, 32, 20
T = 512
NT = S // T
HL = 16
G = 80
F, BF = jnp.float32, jnp.bfloat16


def _dot(a, b):
    return jnp.dot(a, b, preferred_element_type=F)


def _dot_nt(a, b):
    return lax.dot_general(a, b, (((1,), (1,)), ((), ())), preferred_element_type=F)


def _ln(x):
    c = x - jnp.mean(x, -1, keepdims=True)
    return (c * lax.rsqrt(jnp.mean(c * c, -1, keepdims=True) + 1e-5)).astype(BF)


def _sw(m):
    return pltpu.roll(m, 4, 0)


def _fsum(e):
    t = jnp.sum(e, 0)
    return t + _sw(t)


def _softmax_pm(p):
    out = []
    m = jnp.max(p, 0)
    e = jnp.exp(p - jnp.maximum(m, _sw(m))[None])
    out.append((e, 1.0 / _fsum(e)))
    m = jnp.min(p, 0)
    e = jnp.exp(jnp.minimum(m, _sw(m))[None] - p)
    out.append((e, 1.0 / _fsum(e)))
    return out


def _kern(x0h, awqkvh, awoh, bwqkvh, wphih, bwoh, out,
          x0, awqkv, awo, bwqkv, wphi, bwo, sem, osem, tmp,
          x, wa, woa, wbt, wob, qE, qO, kE, kO, vE, vO, pE, pO, kv, zacc, kvb, zb):
    cp = [pltpu.make_async_copy(a, b, sem.at[i]) for i, (a, b) in enumerate(
        ((awqkvh, awqkv), (awoh, awo), (x0h, x0), (bwqkvh, bwqkv), (wphih, wphi), (bwoh, bwo)))]
    for d in cp:
        d.start()
    r = lax.broadcasted_iota(jnp.int32, (D, D), 0)
    c = lax.broadcasted_iota(jnp.int32, (D, D), 1)
    pa = (r == (c & 31) * DH + (c >> 5)).astype(BF)
    cp[0].wait()
    for j in range(3):
        w = _dot(awqkv[:, j * D:(j + 1) * D], pa)
        wa[:, j * D:(j + 1) * D] = w.astype(BF)
    cp[1].wait()
    for ch in range(5):
        tmp[...] = awo[:, ch * 128:(ch + 1) * 128].astype(F)
        for dd in range(DH):
            woa[dd * H:(dd + 1) * H, ch * 128:(ch + 1) * 128] = tmp[pl.ds(dd, H, stride=DH), :].astype(BF)
    for d in cp[2:]:
        d.wait()
    wt = wphi[...].astype(F)
    s8 = lax.broadcasted_iota(jnp.int32, (8, D), 0) < 4
    wrep = jnp.concatenate(
        [jnp.where(s8, jnp.broadcast_to(wt[2 * i:2 * i + 1], (8, D)),
                   jnp.broadcast_to(wt[2 * i + 1:2 * i + 2], (8, D))) for i in range(DH // 2)], 0)
    rg = lax.broadcasted_iota(jnp.int32, (G, 256), 0)
    for g in range(8):
        cb = 128 * min(G * g // 128, 3)
        cg = lax.broadcasted_iota(jnp.int32, (G, 256), 1) + cb
        h0 = (g * 4 + (rg & 3)) * DH
        pbt = (cg == h0 + (rg >> 2)).astype(BF)
        bdt = jnp.where((cg >= h0) & (cg < h0 + DH),
                        wrep[:, cb:cb + 256], 0.0).astype(BF)
        for j, (m_, o) in enumerate(((bdt, D), (pbt, 2 * D), (bdt, 0))):
            wbt[j * D + g * G:j * D + (g + 1) * G, :] = _dot_nt(
                m_, bwqkv[:, o + cb:o + cb + 256]).astype(BF)
        wob[g * G:(g + 1) * G, :] = _dot(pbt, bwo[cb:cb + 256, :]).astype(BF)
    x[...] = x0[...].astype(F)

    buf = ((qE, kE, vE, pE), (qO, kO, vO, pO))

    def rows(s):
        return pl.ds(s * T if isinstance(s, int) else pl.multiple_of(s * T, T), T)

    def a1(s, par):
        q_, k_, v_, _ = buf[par]
        y = _dot(_ln(x[rows(s), :]), wa[...])
        for ch in range(5):
            q_[ch] = y[:, ch * 128:(ch + 1) * 128] * DH ** -0.5
            k_[ch, HL:, :] = y[:, D + ch * 128:D + (ch + 1) * 128]
            v_[ch, HL:, :] = y[:, 2 * D + ch * 128:2 * D + (ch + 1) * 128]

    C = 128

    def a2(s, par):
        q_, k_, v_, _ = buf[par]
        os_ = []
        for r0 in range(0, T, C):
            q = [q_[ch, r0:r0 + C, :] for ch in range(5)]
            pos = s * T + r0 + lax.broadcasted_iota(jnp.int32, (C, 128), 0)
            ls = []
            for w in range(8):
                t = [q[ch] * k_[ch, pl.ds(r0 + HL - 2 * w, C), :] for ch in range(5)]
                l = (t[0] + t[1]) + (t[2] + t[3]) + t[4]
                l = l + pltpu.roll(l, 64, 1)
                l = l + pltpu.roll(l, 32, 1)
                ls.append(l if w == 0 else jnp.where(pos >= 2 * w, l, -1e9))
            m = ls[0]
            for l in ls[1:]:
                m = jnp.maximum(m, l)
            e = [jnp.exp(l - m) for l in ls]
            z = e[0]
            for t in e[1:]:
                z = z + t
            rz = 1.0 / z
            o = []
            for ch in range(5):
                a = e[0] * v_[ch, pl.ds(r0 + HL, C), :]
                for w in range(1, 8):
                    a = a + e[w] * v_[ch, pl.ds(r0 + HL - 2 * w, C), :]
                o.append((a * rz).astype(BF))
            os_.append(jnp.concatenate(o, 1))
        xn = x[rows(s), :] + _dot(jnp.concatenate(os_, 0), woa[...])
        x[rows(s), :] = xn
        return xn

    def halo(par):
        for ch in range(5):
            for i in (1, 2):
                buf[par][i][ch, 0:HL, :] = buf[1 - par][i][ch, T:T + HL, :]

    def b1(xt):
        xn = _ln(xt)
        pv = _dot_nt(wbt[0:2 * D], xn)
        for g in range(8):
            p = pv[g * G:(g + 1) * G].reshape(DH // 2, 8, T)
            vt = pv[D + g * G:D + (g + 1) * G].astype(BF)
            ph = []
            for j, (e, rs) in enumerate(_softmax_pm(p)):
                f = (e * rs[None]).reshape(G, T)
                zs = f[:, 0:128]
                for u in range(128, T, 128):
                    zs = zs + f[:, u:u + 128]
                zacc[g, j * G:(j + 1) * G, :] += zs
                ph.append(f.astype(BF))
            kv[g] += _dot_nt(vt, jnp.concatenate(ph, 0))

    def step_x(s, par, nxt=True):
        halo(par)
        if nxt:
            a1(s + 1, 1 - par)
        b1(a2(s, par))

    def ocp(s):
        return pltpu.make_async_copy(x0.at[rows(s)], out.at[rows(s)], osem.at[s])

    def b2a(s, par):
        buf[par][3][...] = _dot_nt(wbt[2 * D:], _ln(x[rows(s), :]))

    def b2b(s, par):
        pr = buf[par][3]
        ot = []
        for g in range(8):
            p = pr[g * G:(g + 1) * G, :].reshape(DH // 2, 8, T)
            ph, den = [], None
            for j, (e, rs) in enumerate(_softmax_pm(p)):
                z = zb[g, j * G:(j + 1) * G, :]
                z = jnp.concatenate([z] * (T // 128), 1).reshape(DH // 2, 8, T)
                t = jnp.sum(e * z, 0) * rs
                den = t if den is None else den + t
                ph.append((e * rs[None]).reshape(G, T).astype(BF))
            num = _dot(kvb[g], jnp.concatenate(ph, 0))
            rd = 1.0 / (den + _sw(den) + 1e-6)
            ot.append((num.reshape(DH // 2, 8, T) * rd[None]).reshape(G, T))
        o = jnp.concatenate(ot, 0).T.astype(BF)
        xn = x[rows(s), :] + _dot(o, wob[...])
        x[rows(s), :] = xn
        x0[rows(s), :] = xn.astype(BF)
        ocp(s).start()

    def step_y(s, par, nxt=True):
        if nxt:
            b2a(s + 1, 1 - par)
        b2b(s, par)

    def pipeline(step):
        def two(j, _):
            step(2 * j, 0)
            step(2 * j + 1, 1)
            return 0
        for j in range(NT // 2 - 1):
            two(j, 0)
        step(NT - 2, 0)
        step(NT - 1, 1, False)

    def pair(_i, _):
        for ch in range(5):
            kO[ch, T:T + HL, :] = jnp.zeros((HL, 128), F)
            vO[ch, T:T + HL, :] = jnp.zeros((HL, 128), F)
        kv[...] = jnp.zeros(kv.shape, F)
        zacc[...] = jnp.zeros(zacc.shape, F)
        a1(0, 0)
        pipeline(step_x)
        rr = lax.broadcasted_iota(jnp.int32, (G, 2 * G), 0)
        cc = lax.broadcasted_iota(jnp.int32, (G, 2 * G), 1)
        for g in range(8):
            kvb[g] = jnp.where((rr & 3) == (cc & 3), kv[g], 0.0).astype(BF)
            zb[g] = jnp.broadcast_to(jnp.sum(zacc[g], 1, keepdims=True), (2 * G, 128))
        b2a(0, 0)
        pipeline(step_y)
        for s in range(NT):
            ocp(s).wait()
        return 0

    lax.fori_loop(0, 2, pair, 0)


@jax.jit
def pallas_interleave_layers__sliding_local_dilated__linear_kernel_hedgehog__prompt_kernel(
        A_x, A_wqkv, A_wo, B_x, B_wqkv, B_w_phi, B_wo):
    wphi = B_w_phi.transpose(2, 0, 1).reshape(DH, D)
    vm = pltpu.VMEM
    o = pl.pallas_call(
        _kern,
        out_specs=pl.BlockSpec(memory_space=pl.ANY),
        out_shape=jax.ShapeDtypeStruct((S, D), BF),
        in_specs=[pl.BlockSpec(memory_space=pl.ANY)] * 6,
        scratch_shapes=[vm((S, D), BF), vm((D, 3 * D), BF), vm((D, D), BF), vm((D, 3 * D), BF),
                        vm((DH, D), BF), vm((D, D), BF), pltpu.SemaphoreType.DMA((6,)), pltpu.SemaphoreType.DMA((NT,)), vm((D, 128), F),
                        vm((S, D), F), vm((D, 3 * D), BF), vm((D, D), BF),
                        vm((3 * D, D), BF), vm((D, D), BF)]
        + [vm((5, T, 128), F)] * 2 + [vm((5, T + HL, 128), F)] * 4 + [vm((D, T), F)] * 2
        + [vm((8, G, 2 * G), F), vm((8, 2 * G, 128), F),
           vm((8, G, 2 * G), BF), vm((8, 2 * G, 128), F)],
        compiler_params=pltpu.CompilerParams(vmem_limit_bytes=100 << 20),
    )(A_x.reshape(S, D), A_wqkv, A_wo, B_wqkv, wphi, B_wo)
    return o.reshape(1, S, D)
```
